```python
import jax
import jax.numpy as jnp

def _softmax(x, axis=-1):
    return jax.nn.softmax(x, axis=axis)
def _gelu(x):
    return jax.nn.gelu(x, approximate=True)
def _silu(x):
    return jax.nn.silu(x)
def _sigmoid(x):
    return jax.nn.sigmoid(x)
def _layernorm(x, axis=-1, eps=1e-5):
    m = jnp.mean(x, axis=axis, keepdims=True)
    v = jnp.var(x, axis=axis, keepdims=True)
    return (x - m) / jnp.sqrt(v + eps)
def _scatter_add(tgt, idx, src, axis=0):
    return tgt.at[idx].add(src)
def _segment_sum(src, seg, n):
    return jax.ops.segment_sum(src, seg, n)
class _Rng:
    def __init__(self, key):
        self._k = key
    def _next(self):
        self._k, sub = jax.random.split(self._k)
        return sub
    def normal(self, shape):
        return jax.random.normal(self._next(), shape, dtype=jnp.bfloat16)
    def randint(self, lo, hi, shape):
        return jax.random.randint(self._next(), shape, lo, hi, dtype=jnp.int32)
    def uniform(self, shape, lo=0.0, hi=1.0):
        return jax.random.uniform(self._next(), shape, jnp.bfloat16, lo, hi)
    def permutation(self, n):
        return jax.random.permutation(self._next(), n)


kernel_name = 'recurrent_scan__linear_kernel_hedgehog__dense_activation_relu__prompt'

def _fwd_setup_inputs():
    _rng = _Rng(jax.random.key(int.from_bytes(__import__("os").urandom(4), "little")))
    _w = (lambda a: (lambda t: t.astype(jnp.bfloat16) if jnp.issubdtype(t.dtype, jnp.floating) else t)(jnp.asarray(a)))
    def _A_setup():
        B, S, D, H = 1, 2048, 1024, 32
        Dh = D // H
        return {
            "x": _w((lambda *s: _rng.normal(s) * 0.05)(B, S, D)),
            "wqkv": _w((lambda *s: _rng.normal(s) * 0.05)(D, 3 * D)),
            "w_phi": _w((lambda *s: _rng.normal(s) * 0.05)(H, Dh, Dh) * (Dh ** -0.5)),
            "wo": _w((lambda *s: _rng.normal(s) * 0.05)(D, D)),
        }
    _A_in = _A_setup()

    def _B_setup():
        B, S, D, Dff = 1, 2048, 1024, 3584
        return {
            "x": _w((lambda *s: _rng.normal(s) * 0.05)(B, S, D)),
            "w1": _w((lambda *s: _rng.normal(s) * 0.05)(D, Dff)),
            "w2": _w((lambda *s: _rng.normal(s) * 0.05)(Dff, D)),
        }
    _B_in = _B_setup()

    return {
        "A_x": _A_in["x"],
        "A_wqkv": _A_in["wqkv"],
        "A_w_phi": _A_in["w_phi"],
        "A_wo": _A_in["wo"],
        "B_x": _B_in["x"],
        "B_w1": _B_in["w1"],
        "B_w2": _B_in["w2"],
    }

def _fwd_reference(A_x, A_wqkv, A_w_phi, A_wo, B_x, B_w1, B_w2):
    def _A_ref(x, wqkv, w_phi, wo):
        B, S, D = x.shape
        H = 32; Dh = D // H
        qkv = (lambda x, *d: x.transpose(*d))((x @ wqkv).reshape(B, S, 3, H, Dh), 2, 0, 3, 1, 4)
        q, k, v = qkv[0], qkv[1], qkv[2]
        pq = jnp.einsum("bhsd,hdf->bhsf", q, w_phi)
        pk = jnp.einsum("bhsd,hdf->bhsf", k, w_phi)
        phi_q = jnp.concatenate([_softmax(pq, axis=-1), _softmax(-pq, axis=-1)], axis=-1)
        phi_k = jnp.concatenate([_softmax(pk, axis=-1), _softmax(-pk, axis=-1)], axis=-1)
        kv = jnp.einsum("bhsf,bhsd->bhfd", phi_k, v)
        z  = jnp.einsum("bhsf->bhf", phi_k)
        num = jnp.einsum("bhqf,bhfd->bhqd", phi_q, kv)
        den = jnp.einsum("bhqf,bhf->bhq", phi_q, z)[..., None] + 1e-6
        o = num / den
        return (lambda x, *d: x.transpose(*d))(o, 0, 2, 1, 3).reshape(B, S, D) @ wo

    def _B_ref(x, w1, w2):
        h = jnp.einsum("bsd,df->bsf", x, w1)
        zero = jnp.zeros_like(h)
        h = jnp.maximum(h, zero)
        return jnp.einsum("bsf,fd->bsd", h, w2)

    x = A_x
    xn = _layernorm(x, axis=-1)
    s = _A_ref(xn, A_wqkv, A_w_phi, A_wo)
    g = _silu(_B_ref(xn, B_w1, B_w2))
    return x + s * g


def setup_inputs():
    _inp = _fwd_setup_inputs()
    _gk = jax.random.fold_in(jax.random.key(int.from_bytes(__import__("os").urandom(4), "little")), 2**31 - 1)
    _shapes = [[1, 2048, 1024]]
    _dtypes = ['bfloat16']
    _gks = jax.random.split(_gk, len(_shapes))
    _gs = [jax.random.normal(k, s, dtype=jnp.dtype(d)) * 0.05 for k, s, d in zip(_gks, _shapes, _dtypes)]
    _inp["grad_out"] = _gs[0]
    return _inp

def reference(A_x, A_wqkv, A_w_phi, A_wo, B_w1, B_w2, B_x, grad_out):
    _const = dict(B_x=B_x)
    def _f(*_d):
        return _fwd_reference(**{'A_x': _d[0], 'A_wqkv': _d[1], 'A_w_phi': _d[2], 'A_wo': _d[3], 'B_w1': _d[4], 'B_w2': _d[5], **_const})
    _out, _vjp = jax.vjp(_f, A_x, A_wqkv, A_w_phi, A_wo, B_w1, B_w2)
    _grads = _vjp(grad_out)
    _out0 = jnp.asarray(_out)
    return (_out0, *[jnp.asarray(_g) for _g in _grads])
```

```python
import jax
import jax.numpy as jnp
import jax.experimental.pallas as pl
import jax.experimental.pallas.tpu as pltpu

S = 2048
D = 1024
H = 32
DH = 32
DFF = 3584
NG = 8
EXT = 80
F32 = jnp.float32
BF16 = jnp.bfloat16
U32 = jnp.uint32

XCH = 256
NXC = S // XCH
W1T = 512
NW1 = DFF // W1T
TB = 256
NB = S // TB
TF = 256
NF = DFF // TF


def _nn(a, b):
    return jax.lax.dot_general(a, b, (((1,), (0,)), ((), ())), preferred_element_type=F32)


def _nt(a, b):
    return jax.lax.dot_general(a, b, (((1,), (1,)), ((), ())), preferred_element_type=F32)


def _tn(a, b):
    return jax.lax.dot_general(a, b, (((0,), (0,)), ((), ())), preferred_element_type=F32)


def _rows(r0, n):
    if isinstance(r0, int):
        return slice(r0 // 2, (r0 + n) // 2)
    return pl.ds(pl.multiple_of(r0 // 2, 8), n // 2)


def _ld(ref, r0, n, cols=slice(None)):
    return pltpu.bitcast(ref[_rows(r0, n), cols], BF16)


def _st(ref, r0, val, cols=slice(None)):
    ref[_rows(r0, val.shape[0]), cols] = pltpu.bitcast(val.astype(BF16), U32)


def _dual_softmax(p):
    c = p.shape[1]
    p3 = p.reshape(2, DH, c)
    mx = jnp.max(p3, axis=1, keepdims=True)
    mn = jnp.min(p3, axis=1, keepdims=True)
    ep = jnp.exp(p3 - mx)
    en = jnp.exp(mn - p3)
    rp = 1.0 / jnp.sum(ep, axis=1, keepdims=True)
    rn = 1.0 / jnp.sum(en, axis=1, keepdims=True)
    yp = ep * rp
    yn = en * rn
    return jnp.concatenate([yp.reshape(64, c), yn.reshape(64, c)], axis=0)


def _dual_softmax_bwd(y, dy):
    c = y.shape[1]
    y4 = y.reshape(4, DH, c)
    dy4 = dy.reshape(4, DH, c)
    t = jnp.sum(y4 * dy4, axis=1, keepdims=True)
    r = (y4 * (dy4 - t)).reshape(128, c)
    return r[:64] - r[64:]


def _kernel(x_hbm, wqkv_hbm, wphi_hbm, wo_hbm, w1_hbm, w2_hbm, go_hbm,
            out_hbm, dx_hbm, dwqkv_hbm, dwphi_hbm, dwo_hbm, dw1_hbm, dw2_hbm,
            x_v, go_v, wqkv_v, wphi_v, wo_v, w1_v, w2_v,
            xn_v, xnt_v, rstd_v, h_v, g_v, gd_v, ds_v, wt_v, bd_v, bdt_v, dpt_v, ot_v,
            phik_v, phiq_v, vext_v, dot_v, stage_v, stat_v,
            st_dw1, st_dw2, st_dwqkv, st_dwo, st_dwphi,
            x_sems, w1_sems, in_sems, dx_sems, misc_sems):

    def x_copy(i):
        return pltpu.make_async_copy(x_hbm.at[pl.ds(i * XCH, XCH), :], x_v.at[pl.ds(i * XCH, XCH), :], x_sems.at[i])

    def w1_copy(i):
        return pltpu.make_async_copy(w1_hbm.at[:, pl.ds(i * W1T, W1T)], w1_v.at[:, pl.ds(i * W1T, W1T)], w1_sems.at[i])

    def w1_half(k):
        hw = W1T // 2
        return pltpu.make_async_copy(w1_hbm.at[:, pl.ds(k * hw, hw)], w1_v.at[:, pl.ds(k * hw, hw)], in_sems.at[5 + k])

    x_copy(0).start()
    w1_half(0).start()
    in_copies = [
        pltpu.make_async_copy(w2_hbm, w2_v, in_sems.at[0]),
        pltpu.make_async_copy(go_hbm, go_v, in_sems.at[1]),
        pltpu.make_async_copy(wqkv_hbm, wqkv_v, in_sems.at[2]),
        pltpu.make_async_copy(wphi_hbm, wphi_v, in_sems.at[3]),
        pltpu.make_async_copy(wo_hbm, wo_v, in_sems.at[4]),
    ]

    def relu(hp):
        return jnp.where(hp > 0, hp, jnp.where(hp == 0, 0.0, -0.0))

    def layernorm(i):
        RB = 16
        for k in range(XCH // RB):
            r0 = i * XCH + k * RB
            xf = x_v[r0:r0 + RB, :].astype(F32)
            m = jnp.mean(xf, axis=1, keepdims=True)
            xc = xf - m
            var = jnp.mean(xc * xc, axis=1, keepdims=True)
            rstd = 1.0 / jnp.sqrt(var + 1e-5)
            _st(xn_v, r0, xc * rstd)
            rstd_v[r0:r0 + RB, :] = jnp.broadcast_to(rstd, (RB, 128))

    hw = W1T // 2
    x_copy(0).wait()
    w1_half(1).start()
    x_copy(1).start()
    layernorm(0)
    w1_half(0).wait()
    _st(h_v, 0, relu(_nn(_ld(xn_v, 0, XCH), w1_v[:, 0:hw])), slice(0, hw))
    w1_half(1).wait()
    x_copy(1).wait()
    for i in range(2, NXC):
        x_copy(i).start()
    _st(h_v, 0, relu(_nn(_ld(xn_v, 0, XCH), w1_v[:, hw:W1T])), slice(hw, W1T))
    layernorm(1)
    waits = {1: (2,), 2: (3, 4), 4: (5, 6, 7)}
    for i in range(1, NXC):
        for j in waits.get(i, ()):
            x_copy(j).wait()
        if i == 4:
            w1_copy(1).start()
        _st(h_v, i * XCH, relu(_nn(_ld(xn_v, i * XCH, XCH), w1_v[:, 0:W1T])), slice(0, W1T))
        if i + 1 < NXC:
            layernorm(i + 1)

    for i in range(2, NW1):
        w1_copy(i).start()
    for c in in_copies:
        c.start()

    def h_body(i, _):
        f0 = pl.multiple_of(i * W1T, W1T)
        w1_copy(i).wait()
        _st(h_v, 0, relu(_nn(_ld(xn_v, 0, S), w1_v[:, pl.ds(f0, W1T)])), pl.ds(f0, W1T))
        return 0

    jax.lax.fori_loop(1, NW1, h_body, 0)

    for c in in_copies:
        c.wait()

    row128 = jax.lax.broadcasted_iota(jnp.int32, (128, 128), 0)
    col128 = jax.lax.broadcasted_iota(jnp.int32, (128, 128), 1)
    bdmask = (row128 // DH) == (col128 // DH)
    rep = jnp.where(jax.lax.broadcasted_iota(jnp.int32, (DH, 128), 0)
                    == jax.lax.broadcasted_iota(jnp.int32, (DH, 128), 1) % DH, 1.0, 0.0).astype(BF16)

    for g in range(NG):
        wp = wphi_v[g * 128:(g + 1) * 128, :]
        bd = jnp.where(bdmask, _nn(wp, rep), 0.0)
        _st(bd_v, g * 128, bd)
        _st(bdt_v, g * 128, bd.T)

    TB2 = 2 * TB

    def b_body(i, _):
        r0 = pl.multiple_of(i * TB2, TB2)
        b = _nn(_ld(h_v, r0, TB2), w2_v[...])
        sig = jax.nn.sigmoid(b)
        g = b * sig
        gof = go_v[pl.ds(r0, TB2), :].astype(F32)
        _st(g_v, r0, g)
        _st(gd_v, r0, gof * (sig + g * (1.0 - sig)))
        _st(ds_v, r0, gof * g)
        for k in range(2):
            c0 = pl.multiple_of((2 * i + k) * 128, 128)
            w0 = pl.multiple_of((2 * i + k) * 384, 128)
            bdt = _ld(bdt_v, c0, 128)
            _st(wt_v, w0, _nt(bdt, wqkv_v[:, pl.ds(c0, 128)]))
            _st(wt_v, w0 + 128, _nt(bdt, wqkv_v[:, pl.ds(D + c0, 128)]))
            _st(wt_v, w0 + 256, wqkv_v[:, pl.ds(2 * D + c0, 128)].T)
        _st(xnt_v, 0, _ld(xn_v, r0, TB2).T, pl.ds(r0, TB2))
        return 0

    jax.lax.fori_loop(0, NB // 2, b_body, 0)

    er = jax.lax.broadcasted_iota(jnp.int32, (EXT, 128), 0)
    ec = jax.lax.broadcasted_iota(jnp.int32, (EXT, 128), 1)
    ec_head = (ec % 64) // DH
    er_head = jnp.where(er < 64, er // DH, er - 64)
    ext_mask = jnp.logical_and(er < 66, er_head == ec_head)
    _st(vext_v, 64, jnp.where(jax.lax.broadcasted_iota(jnp.int32, (16, S), 0) == 0, 1.0, 0.0))

    def pair(rq, ro, ro_next):
        wt = jnp.concatenate([_ld(wt_v, rq, 64), _ld(wt_v, rq + 128, 64), _ld(wt_v, rq + 256, 64)], axis=0)
        pt = _nn(wt, _ld(xnt_v, 0, D))
        _st(phiq_v, 0, _dual_softmax(pt[0:64]))
        _st(phik_v, 0, _dual_softmax(pt[64:128]))
        _st(vext_v, 0, pt[128:192])
        kvz = _nt(_ld(vext_v, 0, EXT), _ld(phik_v, 0, 128))
        zrow = kvz[64:65, :]
        lhs = jnp.where(er < 64, kvz, zrow)
        lhs = jnp.where(ext_mask, lhs, 0.0).astype(BF16)
        nd = _nn(lhs, _ld(phiq_v, 0, 128))
        do3 = dot_v[...].reshape(2, DH, S)
        den = nd[64:66, :] + 1e-6
        rden = (1.0 / den).reshape(2, 1, S)
        o3 = nd[0:64, :].reshape(2, DH, S) * rden
        dnum = do3 * rden
        dden = -jnp.sum(dnum * o3, axis=1)
        _st(ot_v, ro, o3.reshape(64, S))
        dn = jnp.concatenate([dnum.reshape(64, S), dden, jnp.zeros((EXT - 66, S), F32)], axis=0)
        dnb = dn.astype(BF16)
        dkvz = _nt(dnb, _ld(phiq_v, 0, 128))
        dphiq = _tn(lhs, dnb)
        _st(dpt_v, rq, _dual_softmax_bwd(_ld(phiq_v, 0, 128).astype(F32), dphiq))
        dkvz = jnp.where(ext_mask, dkvz, 0.0)
        dz = dkvz[64:65, :] + dkvz[65:66, :]
        mm = jnp.where(er < 64, dkvz, jnp.where(er == 64, dz, 0.0)).astype(BF16)
        _st(dpt_v, rq + 256, _nn(mm[0:64, :], _ld(phik_v, 0, 128)))
        dphik = _tn(mm, _ld(vext_v, 0, EXT))
        _st(dpt_v, rq + 128, _dual_softmax_bwd(_ld(phik_v, 0, 128).astype(F32), dphik))
        if ro_next is not None:
            dot_v[...] = _nt(wo_v[pl.ds(ro_next, 64), :], _ld(ds_v, 0, S))

    dot_v[...] = _nt(wo_v[0:64, :], _ld(ds_v, 0, S))

    def pair_body(g, _):
        rq = pl.multiple_of(g * 384, 128)
        ro = pl.multiple_of(g * 128, 128)
        pair(rq, ro, ro + 64)
        pair(rq + 64, ro + 64, ro + 128)
        return 0

    jax.lax.fori_loop(0, NG - 1, pair_body, 0)
    pair((NG - 1) * 384, (NG - 1) * 128, (NG - 1) * 128 + 64)
    pair((NG - 1) * 384 + 64, (NG - 1) * 128 + 64, None)

    def out_body(i, _):
        r0 = pl.multiple_of(i * TB, TB)
        c0 = pl.multiple_of(i * 128, 128)
        w0 = pl.multiple_of(i * 384, 128)
        st_dwo[pl.ds(c0, 128), :] = _nn(_ld(ot_v, c0, 128), _ld(ds_v, 0, S)).astype(BF16)
        gg = _nt(_ld(xnt_v, 0, D), _ld(dpt_v, w0, 384)).astype(BF16)
        s = _tn(_ld(ot_v, 0, D, pl.ds(r0, TB)), wo_v[...])
        x_v[pl.ds(r0, TB), :] = (x_v[pl.ds(r0, TB), :].astype(F32)
                                 + s * _ld(g_v, r0, TB).astype(F32)).astype(BF16)
        _st(gd_v, r0, s * _ld(gd_v, r0, TB).astype(F32))
        bd = _ld(bd_v, c0, 128)
        gq = gg[:, 0:128]
        gk = gg[:, 128:256]
        st_dwqkv[:, pl.ds(c0, 128)] = _nt(gq, bd).astype(BF16)
        st_dwqkv[:, pl.ds(D + c0, 128)] = _nt(gk, bd).astype(BF16)
        st_dwqkv[:, pl.ds(2 * D + c0, 128)] = gg[:, 256:384]
        dbd = _tn(wqkv_v[:, pl.ds(c0, 128)], gq) + _tn(wqkv_v[:, pl.ds(D + c0, 128)], gk)
        dbd = jnp.where(bdmask, dbd, 0.0).astype(BF16)
        st_dwphi[pl.ds(c0, 128), :] = _nt(dbd, rep).astype(BF16)
        return 0

    jax.lax.fori_loop(0, NB, out_body, 0)
    out_copies = [
        pltpu.make_async_copy(st_dwphi, dwphi_hbm, misc_sems.at[0]),
        pltpu.make_async_copy(x_v, out_hbm, misc_sems.at[1]),
        pltpu.make_async_copy(st_dwo, dwo_hbm, misc_sems.at[2]),
        pltpu.make_async_copy(st_dwqkv, dwqkv_hbm, misc_sems.at[3]),
        pltpu.make_async_copy(st_dw1, dw1_hbm, misc_sems.at[4]),
        pltpu.make_async_copy(st_dw2, dw2_hbm, misc_sems.at[5]),
    ]
    for c in out_copies[:4]:
        c.start()

    def mb_body(i, _):
        f0 = pl.multiple_of(i * TF, TF)
        db = _ld(gd_v, 0, S)
        hh = _ld(h_v, 0, S, pl.ds(f0, TF))
        dh = _nt(db, w2_v[pl.ds(f0, TF), :])
        hf = hh.astype(F32)
        bits = jax.lax.bitcast_convert_type(hf, jnp.int32)
        dhp = jnp.where(hf > 0, dh, jnp.where(bits == 0, 0.5 * dh, 0.0)).astype(BF16)
        st_dw2[pl.ds(f0, TF), :] = _tn(hh, db).astype(BF16)
        _st(h_v, 0, dhp, pl.ds(f0, TF))
        st_dw1[:, pl.ds(f0, TF)] = _nn(_ld(xnt_v, 0, D), dhp).astype(BF16)
        return 0

    jax.lax.fori_loop(0, NF, mb_body, 0)
    for c in out_copies[4:]:
        c.start()

    def dx_copy(i):
        return pltpu.make_async_copy(x_v.at[pl.ds(i * TB, TB), :], dx_hbm.at[pl.ds(i * TB, TB), :], dx_sems.at[i])

    def ln_bwd(r0, cur):
        rows = pl.ds(r0, TB)
        for c in range(D // 128):
            cs = slice(c * 128, (c + 1) * 128)
            m1 = stat_v[:, 0:128]
            m2 = stat_v[:, 128:256]
            rstd = rstd_v[rows, :]
            xn = _ld(xn_v, r0, TB, cs).astype(F32)
            x_v[rows, cs] = (go_v[rows, cs].astype(F32) + rstd * (stage_v[:, cs] - m1 - xn * m2)).astype(BF16)
            if cur is not None:
                stage_v[:, cs] = cur[:, cs]

    out_copies[1].wait()
    stage_v[...] = jnp.zeros_like(stage_v)
    stat_v[...] = jnp.zeros_like(stat_v)

    def dx_body(i, _):
        r0 = pl.multiple_of(i * TB, TB)
        dxn = _tn(_ld(dpt_v, 0, 3 * D, pl.ds(r0, TB)), _ld(wt_v, 0, 3 * D)) + _nt(_ld(h_v, r0, TB), w1_v[...])
        ln_bwd(pl.multiple_of(jnp.maximum(i - 1, 0) * TB, TB), dxn)
        xn = _ld(xn_v, r0, TB).astype(F32)
        stat_v[:, 0:128] = jnp.broadcast_to(jnp.mean(dxn, axis=1, keepdims=True), (TB, 128))
        stat_v[:, 128:256] = jnp.broadcast_to(jnp.mean(dxn * xn, axis=1, keepdims=True), (TB, 128))

        @pl.when(i > 0)
        def _():
            dx_copy(i - 1).start()
        return 0

    jax.lax.fori_loop(0, NB, dx_body, 0)
    ln_bwd((NB - 1) * TB, None)
    dx_copy(NB - 1).start()

    for k, c in enumerate(out_copies):
        if k != 1:
            c.wait()
    for i in range(NB):
        dx_copy(i).wait()


def _packed(rows, cols):
    return pltpu.VMEM((rows // 2, cols), U32)


@jax.jit
def pallas_recurrent_scan__linear_kernel_hedgehog__dense_activation_relu__prompt_kernel(A_x, A_wqkv, A_w_phi, A_wo, B_x, B_w1, B_w2, grad_out):
    x = A_x.reshape(S, D)
    go = grad_out.reshape(S, D)
    wphi = A_w_phi.reshape(H * DH, DH)
    any_spec = pl.BlockSpec(memory_space=pl.ANY)
    out_shape = (
        jax.ShapeDtypeStruct((S, D), BF16),
        jax.ShapeDtypeStruct((S, D), BF16),
        jax.ShapeDtypeStruct((D, 3 * D), BF16),
        jax.ShapeDtypeStruct((H * DH, DH), BF16),
        jax.ShapeDtypeStruct((D, D), BF16),
        jax.ShapeDtypeStruct((D, DFF), BF16),
        jax.ShapeDtypeStruct((DFF, D), BF16),
    )
    scratch = [
        pltpu.VMEM((S, D), BF16),
        pltpu.VMEM((S, D), BF16),
        pltpu.VMEM((D, 3 * D), BF16),
        pltpu.VMEM((H * DH, DH), BF16),
        pltpu.VMEM((D, D), BF16),
        pltpu.VMEM((D, DFF), BF16),
        pltpu.VMEM((DFF, D), BF16),
        _packed(S, D),
        _packed(D, S),
        pltpu.VMEM((S, 128), F32),
        _packed(S, DFF),
        _packed(S, D),
        _packed(S, D),
        _packed(S, D),
        _packed(3 * D, D),
        _packed(D, 128),
        _packed(D, 128),
        _packed(3 * D, S),
        _packed(D, S),
        _packed(128, S),
        _packed(128, S),
        _packed(EXT, S),
        pltpu.VMEM((64, S), F32),
        pltpu.VMEM((TB, D), F32),
        pltpu.VMEM((TB, 256), F32),
        pltpu.VMEM((D, DFF), BF16),
        pltpu.VMEM((DFF, D), BF16),
        pltpu.VMEM((D, 3 * D), BF16),
        pltpu.VMEM((D, D), BF16),
        pltpu.VMEM((H * DH, DH), BF16),
        pltpu.SemaphoreType.DMA((NXC,)),
        pltpu.SemaphoreType.DMA((NW1,)),
        pltpu.SemaphoreType.DMA((7,)),
        pltpu.SemaphoreType.DMA((NB,)),
        pltpu.SemaphoreType.DMA((6,)),
    ]
    outs = pl.pallas_call(
        _kernel,
        out_shape=out_shape,
        in_specs=[any_spec] * 7,
        out_specs=tuple([any_spec] * 7),
        scratch_shapes=scratch,
        compiler_params=pltpu.CompilerParams(vmem_limit_bytes=127 * 2**20),
    )(x, A_wqkv, wphi, A_wo, B_w1, B_w2, go)
    out, dx, dwqkv, dwphi, dwo, dw1, dw2 = outs
    return (out.reshape(1, S, D), dx.reshape(1, S, D), dwqkv, dwphi.reshape(H, DH, DH), dwo, dw1, dw2)
```
